```python
import os as _os
_os.environ.setdefault("JAX_PLATFORMS", "cpu")
import jax
import jax.numpy as jnp

def _softmax(x, axis=-1):
    return jax.nn.softmax(x, axis=axis)
def _gelu(x):
    return jax.nn.gelu(x, approximate=True)
def _silu(x):
    return jax.nn.silu(x)
def _sigmoid(x):
    return jax.nn.sigmoid(x)
def _layernorm(x, axis=-1, eps=1e-5):
    m = jnp.mean(x, axis=axis, keepdims=True)
    v = jnp.var(x, axis=axis, keepdims=True)
    return (x - m) / jnp.sqrt(v + eps)
def _scatter_add(tgt, idx, src, axis=0):
    return tgt.at[idx].add(src)
def _segment_sum(src, seg, n):
    return jax.ops.segment_sum(src, seg, n)
class _Rng:
    def __init__(self, key):
        self._k = key
    def _next(self):
        self._k, sub = jax.random.split(self._k)
        return sub
    def normal(self, shape):
        return jax.random.normal(self._next(), shape, dtype=jnp.bfloat16)
    def randint(self, lo, hi, shape):
        return jax.random.randint(self._next(), shape, lo, hi, dtype=jnp.int32)
    def uniform(self, shape, lo=0.0, hi=1.0):
        return jax.random.uniform(self._next(), shape, jnp.bfloat16, lo, hi)
    def permutation(self, n):
        return jax.random.permutation(self._next(), n)


kernel_name = 'standalone__gqa_block_cached__near_ridge'

def setup_inputs():
    _rng = _Rng(jax.random.key(int.from_bytes(__import__("os").urandom(4), "little")))
    _w = (lambda a: (lambda t: t.astype(jnp.bfloat16) if jnp.issubdtype(t.dtype, jnp.floating) else t)(jnp.asarray(a)))
    B, Sq, D = 16, 128, 576
    Hq, Hkv, Sk, Dh = 32, 16, 1024, 128
    assert Hq % Hkv == 0, (Hq, Hkv)
    return {
        "x": _w((lambda *s: _rng.normal(s) * 0.8)(B, Sq, D)),
        "k_cache": _w((lambda *s: _rng.normal(s) * 0.8)(B, Hkv, Sk, Dh)),
        "v_cache": _w((lambda *s: _rng.normal(s) * 0.05)(B, Hkv, Sk, Dh)),
        "wq": _w((lambda *s: _rng.normal(s) * 0.8)(D, Hq * Dh) * (D ** -0.5)),
        "wo": _w((lambda *s: _rng.normal(s) * 0.05)(Hq * Dh, D) * ((Hq * Dh) ** -0.5)),
    }

def reference(x, k_cache, v_cache, wq, wo):
    B, Sq, D = x.shape
    Hq, Dh = 32, 128
    Hkv = k_cache.shape[1]
    rep = Hq // Hkv
    q = (lambda x, *d: x.transpose(*d))((x @ wq).reshape(B, Sq, Hq, Dh), 0, 2, 1, 3)
    k = jnp.repeat(k_cache, rep, axis=1)
    v = jnp.repeat(v_cache, rep, axis=1)
    scores = jnp.einsum("bhqd,bhkd->bhqk", q, k) * (Dh ** -0.5)
    p = _softmax(scores, axis=-1)
    o = jnp.einsum("bhqk,bhkd->bhqd", p, v)
    return (lambda x, *d: x.transpose(*d))(o, 0, 2, 1, 3).reshape(B, Sq, Hq * Dh) @ wo
```

```python
import functools
import math

import jax
import jax.numpy as jnp
import jax.experimental.pallas as pl
import jax.experimental.pallas.tpu as pltpu

BB = 2
HH = 4


def _softmax_pv(s, v):
    m = jnp.max(s, axis=1, keepdims=True)
    p = jnp.exp2(s - m)
    l = jnp.sum(p, axis=1, keepdims=True)
    o = jnp.dot(p.astype(jnp.bfloat16), v, preferred_element_type=jnp.float32)
    return (o / l).astype(jnp.bfloat16)


def _kernel(xt_ref, k_ref, v_ref, wq_hbm, wot_hbm, out_ref,
            wq_v, wot_v, sems, x_scr, q_scr, o_prev, acc_ref, s_prev, v_prev,
            *, bb, hh, rep, sq, dh, scale, ni, nj):
    i = pl.program_id(0)
    j = pl.program_id(1)
    cols = hh * rep * dh
    c0 = pl.multiple_of(j * cols, cols)
    jp = jnp.where(j == 0, nj - 1, j - 1)
    cp = pl.multiple_of(jp * cols, cols)
    first = jnp.logical_and(i == 0, j == 0)

    def w_copy(src, dst, which, jj, start):
        return pltpu.make_async_copy(src.at[:, pl.ds(start, cols)],
                                     dst.at[:, pl.ds(start, cols)],
                                     sems.at[which, jj])

    def store_o(o, bi, hi):
        for r in range(rep):
            c = (hi * rep + r) * dh
            o_prev[bi, :, c:c + dh] = o[r * sq:(r + 1) * sq, :]

    def o_proj(start):
        return [jax.lax.dot_general(
            wot_v[:, pl.ds(start, cols)], o_prev[bi], (((1,), (1,)), ((), ())),
            preferred_element_type=jnp.float32) for bi in range(bb)]

    @pl.when(first)
    def _():
        for jj in range(nj):
            w_copy(wq_hbm, wq_v, 0, jj, jj * cols).start()
            jo = (jj - 1) % nj
            w_copy(wot_hbm, wot_v, 1, jo, jo * cols).start()
        o_prev[...] = jnp.zeros(o_prev.shape, o_prev.dtype)
        acc_ref[...] = jnp.zeros(acc_ref.shape, acc_ref.dtype)
        s_prev[...] = jnp.zeros(s_prev.shape, s_prev.dtype)
        v_prev[...] = jnp.zeros(v_prev.shape, v_prev.dtype)
        w_copy(wot_hbm, wot_v, 1, nj - 1, (nj - 1) * cols).wait()

    @pl.when(j == 0)
    def _():
        for bi in range(bb):
            x_scr[bi * sq:(bi + 1) * sq, :] = xt_ref[bi].T

    @pl.when(i == 0)
    def _():
        w_copy(wq_hbm, wq_v, 0, j, c0).wait()

    @pl.when(jnp.logical_and(i == 0, j > 0))
    def _():
        w_copy(wot_hbm, wot_v, 1, jp, cp).wait()

    q = jnp.dot(x_scr[...], wq_v[:, pl.ds(c0, cols)], preferred_element_type=jnp.float32)
    q = (q * scale).astype(jnp.bfloat16)
    for bi in range(bb):
        for hi in range(hh):
            for r in range(rep):
                c = (hi * rep + r) * dh
                q_scr[bi, hi, r * sq:(r + 1) * sq, :] = q[bi * sq:(bi + 1) * sq, c:c + dh]

    store_o(_softmax_pv(s_prev[...], v_prev[...]), bb - 1, hh - 1)

    outs = []
    for bi in range(bb):
        for hi in range(hh):
            s = jax.lax.dot_general(q_scr[bi, hi], k_ref[bi, hi], (((1,), (1,)), ((), ())),
                                    preferred_element_type=jnp.float32)
            if bi == bb - 1 and hi == hh - 1:
                s_last = s
            else:
                outs.append(_softmax_pv(s, v_ref[bi, hi]))

    contribs = o_proj(cp)
    for bi in range(bb):
        acc_ref[bi] = jnp.where(j == 1, contribs[bi], acc_ref[bi] + contribs[bi])

    s_prev[...] = s_last
    v_prev[...] = v_ref[bb - 1, hh - 1]
    for n, o in enumerate(outs):
        store_o(o, n // hh, n % hh)

    @pl.when(jnp.logical_and(j == 0, i > 0))
    def _():
        out_ref[...] = acc_ref[...].astype(out_ref.dtype)

    @pl.when(jnp.logical_and(i == ni - 1, j == nj - 1))
    def _():
        store_o(_softmax_pv(s_prev[...], v_prev[...]), bb - 1, hh - 1)
        contribs = o_proj(c0)
        for bi in range(bb):
            out_ref[bi] = (acc_ref[bi] + contribs[bi]).astype(out_ref.dtype)


@jax.jit
def pallas_standalone__gqa_block_cached__near_ridge_kernel(
    x: jax.Array,
    k_cache: jax.Array,
    v_cache: jax.Array,
    wq: jax.Array,
    wo: jax.Array,
):
    B, Sq, D = x.shape
    _, Hkv, Sk, Dh = k_cache.shape
    Hq = wq.shape[1] // Dh
    rep = Hq // Hkv
    bb, hh = BB, HH
    ni, nj = B // bb, Hkv // hh
    scale = (Dh ** -0.5) * math.log2(math.e)
    xt = x.transpose(0, 2, 1)
    wot = wo.T
    kern = functools.partial(_kernel, bb=bb, hh=hh, rep=rep, sq=Sq, dh=Dh, scale=scale,
                             ni=ni, nj=nj)
    out_t = pl.pallas_call(
        kern,
        grid=(ni, nj),
        in_specs=[
            pl.BlockSpec((bb, D, Sq), lambda i, j: (i, 0, 0)),
            pl.BlockSpec((bb, hh, Sk, Dh), lambda i, j: (i, j, 0, 0)),
            pl.BlockSpec((bb, hh, Sk, Dh), lambda i, j: (i, j, 0, 0)),
            pl.BlockSpec(memory_space=pl.ANY),
            pl.BlockSpec(memory_space=pl.ANY),
        ],
        out_specs=pl.BlockSpec(
            (bb, D, Sq),
            lambda i, j: (jnp.where(j == 0, jnp.maximum(i - 1, 0), i), 0, 0)),
        out_shape=jax.ShapeDtypeStruct((B, D, Sq), x.dtype),
        scratch_shapes=[
            pltpu.VMEM((D, Hq * Dh), jnp.bfloat16),
            pltpu.VMEM((D, Hq * Dh), jnp.bfloat16),
            pltpu.SemaphoreType.DMA((2, nj)),
            pltpu.VMEM((bb * Sq, D), jnp.bfloat16),
            pltpu.VMEM((bb, hh, rep * Sq, Dh), jnp.bfloat16),
            pltpu.VMEM((bb, Sq, hh * rep * Dh), jnp.bfloat16),
            pltpu.VMEM((bb, D, Sq), jnp.float32),
            pltpu.VMEM((rep * Sq, Sk), jnp.float32),
            pltpu.VMEM((Sk, Dh), jnp.bfloat16),
        ],
        compiler_params=pltpu.CompilerParams(
            dimension_semantics=("arbitrary", "arbitrary"),
            vmem_limit_bytes=100 * 1024 * 1024,
        ),
    )(xt, k_cache, v_cache, wq, wot)
    return out_t.transpose(0, 2, 1)
```
